```python
import jax
import jax.numpy as jnp

def _softmax(x, axis=-1):
    return jax.nn.softmax(x, axis=axis)

def _gelu(x):
    return jax.nn.gelu(x, approximate=True)

def _silu(x):
    return jax.nn.silu(x)

def _sigmoid(x):
    return jax.nn.sigmoid(x)

def _layernorm(x, axis=-1, eps=1e-05):
    m = jnp.mean(x, axis=axis, keepdims=True)
    v = jnp.var(x, axis=axis, keepdims=True)
    return (x - m) / jnp.sqrt(v + eps)

def _scatter_add(tgt, idx, src, axis=0):
    return tgt.at[idx].add(src)

def _segment_sum(src, seg, n):
    return jax.ops.segment_sum(src, seg, n)

class _Rng:

    def __init__(self, key):
        self._k = key

    def _next(self):
        self._k, sub = jax.random.split(self._k)
        return sub

    def normal(self, shape):
        return jax.random.normal(self._next(), shape, dtype=jnp.bfloat16)

    def randint(self, lo, hi, shape):
        return jax.random.randint(self._next(), shape, lo, hi, dtype=jnp.int32)

    def uniform(self, shape, lo=0.0, hi=1.0):
        return jax.random.uniform(self._next(), shape, jnp.bfloat16, lo, hi)

    def permutation(self, n):
        return jax.random.permutation(self._next(), n)
kernel_name = 'adaLN_cond__grouped_kv_mqa__dense_activation_silu__prompt'

def _fwd_setup_inputs():
    _rng = _Rng(jax.random.key(int.from_bytes(__import__("os").urandom(4), "little")))
    _w = lambda a: (lambda t: t.astype(jnp.bfloat16) if jnp.issubdtype(t.dtype, jnp.floating) else t)(jnp.asarray(a))

    def _A_setup():
        B, S, D, H = (1, 2048, 640, 32)
        Dh = D // H
        return {'x': _w((lambda *s: _rng.normal(s) * 0.05)(B, S, D)), 'wq': _w((lambda *s: _rng.normal(s) * 0.05)(D, H * Dh)), 'wk': _w((lambda *s: _rng.normal(s) * 0.05)(D, Dh)), 'wv': _w((lambda *s: _rng.normal(s) * 0.05)(D, Dh)), 'wo': _w((lambda *s: _rng.normal(s) * 0.05)(H * Dh, D))}
    _A_in = _A_setup()

    def _B_setup():
        B, S, D, F = (1, 2048, 640, 1728)
        return {'x': _w((lambda *s: _rng.normal(s) * 0.05)(B, S, D)), 'w1': _w((lambda *s: _rng.normal(s) * 0.05)(D, F) * D ** (-0.5)), 'w2': _w((lambda *s: _rng.normal(s) * 0.05)(F, D) * F ** (-0.5))}
    _B_in = _B_setup()
    return {'A_x': _A_in['x'], 'A_wq': _A_in['wq'], 'A_wk': _A_in['wk'], 'A_wv': _A_in['wv'], 'A_wo': _A_in['wo'], 'B_x': _B_in['x'], 'B_w1': _B_in['w1'], 'B_w2': _B_in['w2'], 'c': _w((lambda *s: _rng.normal(s) * 0.05)(1, 640)), 'w_mod': _w((lambda *s: _rng.normal(s) * 0.05)(640, 6 * 640) * 640 ** (-0.5))}

def _fwd_reference(A_x, A_wq, A_wk, A_wv, A_wo, B_x, B_w1, B_w2, c, w_mod):

    def _A_ref(x, wq, wk, wv, wo):
        B, S, D = x.shape
        H = 32
        Dh = D // H
        q = (lambda x, *d: x.transpose(*d))((x @ wq).reshape(B, S, H, Dh), 0, 2, 1, 3)
        k = x @ wk
        v = x @ wv
        scores = jnp.einsum('bhqd,bkd->bhqk', q, k) * Dh ** (-0.5)
        p = _softmax(scores, axis=-1)
        o = jnp.einsum('bhqk,bkd->bhqd', p, v)
        return (lambda x, *d: x.transpose(*d))(o, 0, 2, 1, 3).reshape(B, S, H * Dh) @ wo

    def _B_ref(x, w1, w2):
        h = jnp.einsum('bsd,df->bsf', x, w1)
        h = _silu(h)
        out = jnp.einsum('bsf,fd->bsd', h, w2)
        return out
    x = A_x
    mod = (_silu(c) @ w_mod).reshape(c.shape[0], 6, 1, -1)
    sa, ca, ga, sb, cb, gb = (mod[:, 0].copy(), mod[:, 1].copy(), mod[:, 2].copy(), mod[:, 3].copy(), mod[:, 4].copy(), mod[:, 5].copy())
    h = _layernorm(x, axis=-1) * (1 + ca) + sa
    x = x + ga * _A_ref(h, A_wq, A_wk, A_wv, A_wo)
    h = _layernorm(x, axis=-1) * (1 + cb) + sb
    x = x + gb * _B_ref(h, B_w1, B_w2)
    return x

def setup_inputs():
    _inp = _fwd_setup_inputs()
    _gk = jax.random.fold_in(jax.random.key(int.from_bytes(__import__("os").urandom(4), "little")), 2 ** 31 - 1)
    _shapes = [[1, 2048, 640]]
    _dtypes = ['bfloat16']
    _gks = jax.random.split(_gk, len(_shapes))
    _gs = [jax.random.normal(k, s, dtype=jnp.dtype(d)) * 0.05 for k, s, d in zip(_gks, _shapes, _dtypes)]
    _inp['grad_out'] = _gs[0]
    return _inp

def reference(A_x, A_wq, A_wk, A_wv, A_wo, B_w1, B_w2, c, w_mod, B_x, grad_out):
    _const = dict(B_x=B_x)

    def _f(*_d):
        return _fwd_reference(**{'A_x': _d[0], 'A_wq': _d[1], 'A_wk': _d[2], 'A_wv': _d[3], 'A_wo': _d[4], 'B_w1': _d[5], 'B_w2': _d[6], 'c': _d[7], 'w_mod': _d[8], **_const})
    _out, _vjp = jax.vjp(_f, A_x, A_wq, A_wk, A_wv, A_wo, B_w1, B_w2, c, w_mod)
    _grads = _vjp(grad_out)
    _out0 = jnp.asarray(_out)
    return (_out0, *[jnp.asarray(_g) for _g in _grads])
```

```python
import math

import jax
import jax.numpy as jnp
from jax import lax
from jax.experimental import pallas as pl
from jax.experimental.pallas import tpu as pltpu

BF, F32, U32 = jnp.bfloat16, jnp.float32, jnp.uint32
NN = (((1,), (0,)), ((), ()))
NT = (((1,), (1,)), ((), ()))
TN = (((0,), (0,)), ((), ()))

H = 32
DH = 20
BQ = 512
HB = BQ // 2
CK = 128
VG = ((1, 2), (2, 3))
PACE = ((11, 17), (12, 22))
UF = 6
UB = 4
FC = 96
MA = 48
MO = 64
DC = 128
KC = 512
EPS = 1e-5
LANES = 128


def _dot(a, b, dims=NN):
    return lax.dot_general(a, b, dims, preferred_element_type=F32)


def _pack(x):
    return pltpu.bitcast(x.astype(BF), U32)


def _unpack(x):
    return pltpu.bitcast(x, BF)


def _wide(col, n=BQ):
    return lax.concatenate([col] * (n // LANES), 1)


def _fold(x):
    acc = x[:, :LANES]
    for t in range(1, x.shape[1] // LANES):
        acc = acc + x[:, t * LANES:(t + 1) * LANES]
    return acc


def _colsum(x):
    return jnp.sum(x, axis=0, keepdims=True)


def _sigmoid(x):
    return 0.5 * jnp.tanh(0.5 * x) + 0.5


def _rows(n, m):
    return lax.broadcasted_iota(jnp.int32, (n, m), 0)


def _mix(*streams):
    steps = [(k / len(items), n, fn, item)
             for n, (fn, items) in enumerate(streams) for k, item in enumerate(items)]
    for _, _, fn, item in sorted(steps, key=lambda t: t[:2]):
        fn(item)


def _block_sums(x11, x12, x21, x22):
    x11, x12, x21, x22 = (x.astype(F32) for x in (x11, x12, x21, x22))
    return [x11 + x22, x21 + x22, x11 + x12, x21 - x11, x12 - x22]


def _seven(a11, a22, a, b11, b22, b, dims):
    m = [_dot(x, y, dims) for x, y in
         ((a[0], b[0]), (a[1], b11), (a22, b[3]), (a11, b[4]), (a[2], b22), (a[3], b[2]), (a[4], b[1]))]
    return (jnp.concatenate([m[0] + m[2] - m[4] + m[6], m[3] + m[4]], axis=1),
            jnp.concatenate([m[1] + m[2], m[0] - m[1] + m[3] + m[5]], axis=1), m)


class _Split:
    steps = range(0, HB // 2, 16)

    def __init__(self, x, buf, dims):
        self.x, self.buf, self.dims = x, buf, dims

    def prepare(self, r, gate=lambda words: words):
        top, bot = (_unpack(gate(self.x[r0 + r:r0 + r + 16])) for r0 in (0, HB // 2))
        q = [top[:, :HB], top[:, HB:], bot[:, :HB], bot[:, HB:]]
        if self.dims == NT:
            q = [q[0], q[2], q[1], q[3]]
        self.buf[r:r + 16] = _pack(jnp.concatenate(_block_sums(*q), axis=1))

    def __call__(self, top, bot):
        b = [_unpack(self.buf[:, n * HB:(n + 1) * HB]) for n in range(5)]
        b11, b22, rest = _unpack(self.x[:HB // 2, :HB]), _unpack(self.x[HB // 2:HB, HB:]), _unpack(self.x[HB:])
        q = [top[:, :HB], top[:, HB:BQ], bot[:, :HB], bot[:, HB:BQ]]
        t, u, self.products = _seven(q[0], q[3], _block_sums(*q), b11, b22, b, self.dims)
        m = t.shape[0]
        if self.dims == NT:
            e = _dot(jnp.concatenate([top, bot], axis=0), rest, NT)
            return jnp.concatenate([t, e[:m]], axis=1), jnp.concatenate([u, e[m:]], axis=1)
        e = _dot(jnp.concatenate([top[:, BQ:], bot[:, BQ:]], axis=0), rest)
        return t + e[:m], u + e[m:]


def _chunks(n, m):
    return [slice(r, min(r + m, n)) for r in range(0, n, m)]


def _pairs(n, m):
    return [(slice(r, r + m), slice(n // 2 + r, n // 2 + r + m)) for r in range(0, n // 2, m)]


def _join_heads(heads):
    out = []
    for a, b in zip(heads[0::2], heads[1::2]):
        b = pltpu.roll(b, 4, 0)
        out += [a[0:16], jnp.where(_rows(8, a.shape[1]) < 4, a[16:24], b[0:8]), b[8:24]]
    return jnp.concatenate(out, axis=0)


def _head_rows(ref, h):
    r0 = (h // 2) * 2 * DH
    return pltpu.roll(ref[r0 + 16:r0 + 40], DH, 0) if h % 2 else ref[r0:r0 + 24]


def _ds(start, size):
    return pl.ds(start if isinstance(start, int) else pl.multiple_of(start, math.gcd(size, 16)), size)


def _vpu_groups():
    return [(bwd, c, g) for bwd in range(2) for c in range(BQ // CK) for g in range(VG[bwd][c % 2])]


def _table_tiles():
    return len(_vpu_groups()) * DH


def _arena_rows(S):
    per = BQ // LANES
    return [S, S, S // per, S // BQ * _table_tiles() * 8 // per] + [S // BQ * 24] * 4


def _kernel(x_hbm, g_hbm, wq_hbm, wo_hbm, w1t_hbm, w2_hbm, wmod_hbm, wkt_hbm, wvt_hbm, c_hbm,
            out_hbm, dx_hbm, dwq_hbm, dwo_hbm, dw1t_hbm, dw2_hbm, dwmod_hbm, dwkt_hbm, dwvt_hbm, dc_hbm,
            xt, h1t, st1, dx1t, dqt, arena, e_s, ql, ol, modc, dmodc,
            wq, wbuf, dwo_acc, dw1_acc, dw2_acc, g_in, silu_c, wkt_ref, wvt_ref, c_ref, sems):
    S, D = x_hbm.shape
    F = w2_hbm.shape[0]
    NB = S // BQ
    NC = S // CK
    qscale = DH ** -0.5 * math.log2(math.e)
    inv_d = 1.0 / D
    dch, lch = _chunks(D, DC), _chunks(D, LANES)

    views, row = [], 0
    for rows in _arena_rows(S):
        views.append(arena.at[pl.ds(row, rows)])
        row += rows
    s_a, s_b, vk, vkb, kt, vt, dkt, dvt = views

    def tile(n, rows, used=None, lanes=LANES):
        r0, l0 = n // (BQ // LANES) * rows, n % (BQ // LANES) * LANES
        return slice(r0, r0 + (used or rows)), slice(l0, l0 + lanes)

    def half(r):
        return slice(r.start // 2, r.stop // 2)

    def blk(i, r=slice(0, D)):
        return _ds(i * (D // 2) + r.start // 2, (r.stop - r.start) // 2)

    def copy(src, dst, k):
        return pltpu.make_async_copy(src, dst, sems.at[k])

    def accumulate(st, key, x):
        x = jnp.sum(x.reshape(-1, 8, BQ), axis=0)
        st[key] = st[key] + x if key in st else x

    def set_mod(j, w):
        m = _dot(silu_c[0:8], w)
        if j in (1, 4):
            m = m + 1.0
        modc[j] = jnp.broadcast_to(m[0:1], (LANES, D)).T

    def kv_weights():
        zero4 = jnp.zeros((4, D), F32)
        return jnp.concatenate([wvt_ref[...].astype(F32), zero4, wkt_ref[...].astype(F32), zero4], axis=0)

    def g_copy(i):
        return copy(g_hbm.at[_ds(i * BQ, BQ)], g_in, 3)

    wo, w1t, w2 = wbuf.at[pl.ds(0, D)], wbuf.at[pl.ds(D, F)], wbuf.at[pl.ds(D + F, F)]
    mod_in = [copy(wmod_hbm.at[:, pl.ds(j * D, D)], wbuf.at[pl.ds(j * D, D)], 7 + j) for j in range(6)]

    def prologue(x_in, wm, w_gate):
        def x_copy(i):
            return copy(x_hbm.at[_ds(i * BQ, BQ)], x_in.at[i], 7 + i)

        cp_wm = copy(wmod_hbm.at[:, pl.ds(0, 2 * D)], wm, 4)
        cp_gate = copy(wmod_hbm.at[:, pl.ds(5 * D, D)], w_gate, 5)
        cp_wq = copy(wq_hbm, wq, 6)
        small = [copy(wkt_hbm, wkt_ref, 0), copy(wvt_hbm, wvt_ref, 1), copy(c_hbm, c_ref, 2)]
        for cp in small + [cp_wm] + [x_copy(i) for i in range(NB // 2)]:
            cp.start()
        for acc in (dmodc, dwo_acc, dw1_acc, dw2_acc):
            acc[...] = jnp.zeros_like(acc)
        dkt[...] = jnp.zeros(dkt.shape, F32)
        dvt[...] = jnp.zeros(dvt.shape, F32)

        def project(i):
            x_i, h_i = xt.at[blk(i)], h1t.at[blk(i)]
            st = {}
            for r in lch:
                xb = x_in[i, :, r].T
                x_i[half(r)] = pltpu.bitcast(xb, U32)
                accumulate(st, "sum", xb.astype(F32))
            mu = _colsum(st["sum"]) * inv_d
            for r in lch:
                xc = _unpack(x_i[half(r)]).astype(F32) - mu
                accumulate(st, "var", xc * xc)
            rstd = lax.rsqrt(_colsum(st["var"]) * inv_d + EPS)
            st1[i, 0] = jnp.broadcast_to(mu, (8, BQ))
            st1[i, 1] = jnp.broadcast_to(rstd, (8, BQ))
            for r in dch:
                xh = (_unpack(x_i[half(r)]).astype(F32) - mu) * rstd
                h_i[half(r)] = _pack(xh * _wide(modc[1, r]) + _wide(modc[0, r]))
            r24 = _rows(24, BQ)
            p = _dot(kv_weights(), _unpack(h_i[...])).astype(BF).astype(F32)
            v, k = p[0:24], p[24:48]
            kt[_ds(i * 24, 24)] = k
            vt[_ds(i * 24, 24)] = jnp.where(r24 >= DH, 1.0, v)
            v = jnp.where(r24 < DH, v, jnp.where(r24 < DH + 3, -1.0, 0.0))
            t = jnp.concatenate([v, k, jnp.zeros((LANES - 48, BQ), F32)], axis=0).T
            for n in range(BQ // CK):
                vk.at[_ds(i * CK, CK)][tile(n, CK)] = t[n * CK:(n + 1) * CK]
            table = vkb.at[_ds(i * (vkb.shape[0] // NB), vkb.shape[0] // NB)]
            for n, (bwd, c, g) in enumerate(_vpu_groups()):
                r0 = (c + 1) * CK - 8 * (VG[bwd][c % 2] - g)
                for d in range(DH):
                    lane = d if bwd else 24 + d
                    table[tile(n * DH + d, 8)] = jnp.broadcast_to(t[r0:r0 + 8, lane:lane + 1], (8, LANES))

        for cp in small:
            cp.wait()
        cv = c_ref[...].astype(F32)
        csig = _sigmoid(cv)
        silu_c[0:8] = jnp.broadcast_to(cv * csig, (8, D))
        silu_c[8:16] = jnp.broadcast_to(csig * (1.0 + cv * (1.0 - csig)), (8, D))
        cp_wm.wait()
        for cp in [x_copy(i) for i in range(NB // 2, NB)] + [cp_wq, cp_gate, g_copy(0)]:
            cp.start()
        for j in range(2):
            set_mod(j, wm[:, j * D:(j + 1) * D])

        @pl.loop(0, 2)
        def _(n):
            for u in range(NB // 2):
                x_copy(n * (NB // 2) + u).wait()

            for u in range(NB // 2):
                project(n * (NB // 2) + u)

        cp_wq.wait()
        cp_gate.wait()
        set_mod(5, w_gate[...])

    pl.run_scoped(prologue, pltpu.VMEM((NB, BQ, D), BF), pltpu.VMEM((D, 2 * D), BF), pltpu.VMEM((D, D), BF))

    def epilogue(dwq, dx_out, dkv_b):
        GQ = (D - 2 * LANES) // NB
        n_rest = 2

        def mod_copy(j, slot):
            col = j * D if isinstance(j, int) else pl.multiple_of(j * D, LANES)
            return copy(wbuf.at[_ds(slot * D, D)], dwmod_hbm.at[:, pl.ds(col, D)], j)

        def dx_copy(i):
            return copy(dx_out.at[i % 2], dx_hbm.at[_ds(i * BQ, BQ)], 6 + i)

        def dwq_copy(start, size, k):
            return copy(dwq.at[_ds(start, size)], dwq_hbm.at[_ds(start, size)], 6 + NB + k)

        small_out = [copy(wkt_ref, dwkt_hbm, 13), copy(wvt_ref, dwvt_hbm, 14), copy(c_ref, dc_hbm, 15)]

        def run():
            wkv, sc_col, dsc = (modc.at[j] for j in range(2, 5))
            own = _rows(24, BQ) < DH
            for i in range(NB):
                dkv = jnp.concatenate([jnp.where(own, dvt[i * 24:(i + 1) * 24], 0.0),
                                       jnp.where(own, dkt[i * 24:(i + 1) * 24] * math.log(2.0), 0.0)], axis=0)
                dkv_b[i * 24:(i + 1) * 24] = _pack(dkv)
            wkv[...] = jnp.concatenate([kv_weights(), jnp.zeros((LANES - 48, D), F32)], axis=0).T
            sc_col[...] = jnp.broadcast_to(silu_c[0:8][0:1], (LANES, D)).T
            dsc[...] = jnp.zeros_like(dsc)
            def mod_grad(j, slot):
                row, out = _colsum(dmodc[j].T), wbuf.at[_ds(slot * D, D)]
                for r in range(0, D, 32):
                    out[r:r + 32] = (_wide(sc_col[r:r + 32], D) * row).astype(BF)
                mod_copy(j, slot).start()

            def c_grad(j):
                row, w, digests = _colsum(dmodc[j].T), wbuf.at[_ds(j * D, D)], []
                for r in dch:
                    t = dsc[r] + _fold(w[r].astype(F32) * row)
                    dsc[r] = t
                    digests.append(jnp.sum(t.reshape(-1, 8, LANES), axis=0))
                return digests

            def g_wq(start, size, wait=()):
                parts = []
                for i in range(NB):
                    lhs = h1t[_ds(i * (D // 2) + start // 2, size // 2)]
                    for digest in wait[i:i + 1 if i < NB - 1 else None]:
                        last = jnp.where(start < 0, _wide(pltpu.bitcast(digest, U32)), lhs[-8:])
                        lhs = jnp.concatenate([lhs[:-8], last], axis=0)
                    parts.append(_dot(_unpack(lhs), _unpack(dqt[blk(i)]), NT))
                dwq[_ds(start, size)] = sum(parts[1:], parts[0]).astype(BF)
                return parts

            def rows_of_block(i, dwkv):
                @pl.when(i >= 2)
                def _():
                    dx_copy(i - 2).wait()

                x_i, dq_i, dx1_i = (ref.at[blk(i)] for ref in (xt, dqt, dx1t))
                mu, rstd = st1[i, 0, 0:1], st1[i, 1, 0:1]
                st = {}
                wait = c_grad(i + 2)
                mod_grad(i + 2, i + 2)
                for r in _chunks(D, MO):
                    dh1 = _dot(wq[r], _unpack(dq_i[...])) + _dot(wkv[r, :48], _unpack(dkv_b[_ds(i * 24, 24)]))
                    xh = (_unpack(x_i[half(r)]).astype(F32) - mu) * jnp.where(
                        i < 0, _wide(wait[r.start // DC][0:1]), rstd)
                    t = dh1 * xh
                    dmodc[0, r] += _fold(dh1)
                    dmodc[1, r] += _fold(t)
                    ca = _wide(modc[1, r])
                    dy = dh1 * ca
                    s_a[r] = dy
                    s_b[r] = xh
                    accumulate(st, "m1", dy)
                    accumulate(st, "m2", t * ca)
                parts = g_wq(i * GQ, GQ)
                dwkv = dwkv + _dot(_unpack(dkv_b[_ds(i * 24, 24)]), _unpack(h1t[blk(i)]), NT)
                m1, m2 = (_colsum(st[k]) * inv_d for k in ("m1", "m2"))
                for n, r in enumerate(lch):
                    if n > 1:
                        m1, m2 = (jnp.where(i < 0, parts[n - 2][0:1, :BQ], m) for m in (m1, m2))
                    dx = _unpack(dx1_i[half(r)]).astype(F32) + rstd * (s_a[r] - m1 - s_b[r] * m2)
                    dx_out[i % 2, :, r] = dx.astype(BF).T
                dx_copy(i).start()
                return dwkv

            dwkv = lax.fori_loop(0, NB, rows_of_block, jnp.zeros((48, D), F32))
            dwq_copy(0, NB * GQ, n_rest).start()
            wvt_ref[...] = dwkv[0:DH].astype(BF)
            wkt_ref[...] = dwkv[24:24 + DH].astype(BF)
            small_out[0].start()
            small_out[1].start()

            for j in range(2):
                mod_copy(j + 2, j + 2).wait()
            for j in range(2):
                mod_grad(j, j + 2)

            @pl.loop(0, n_rest)
            def _(j):
                g_wq(NB * GQ + j * LANES, LANES, c_grad(j))
                dwq_copy(NB * GQ + j * LANES, LANES, j).start()

            c_ref[...] = (_colsum(dsc[...].T) * silu_c[8:16][0:1]).astype(BF)
            small_out[2].start()

        return run, ([mod_copy(j, j if j > 1 else j + 2) for j in (0, 1, 4, 5)] + [dx_copy(NB - 2), dx_copy(NB - 1)]
                     + [dwq_copy(0, NB * GQ, n_rest)] + small_out
                     + [dwq_copy(NB * GQ + n * LANES, LANES, n) for n in range(n_rest)])

    def main(at, dut, gt, dft, h2t, obt, sum_a, sum_b, sum_c, dwq, dx_out):
        o_out = g_in
        dql = at
        s_s = (s_a, s_b)

        late_in = [copy(wo_hbm, wo, 0), copy(w1t_hbm, w1t, 1), copy(w2_hbm, w2, 2)]
        early_out = [copy(wo, dwo_hbm, 0), copy(w1t, dw1t_hbm, 1), copy(w2, dw2_hbm, 2)]

        def o_copy(i):
            return copy(o_out, out_hbm.at[_ds(i * BQ, BQ)], 6)

        def head(ref, h):
            return ref.at[_ds(h * 24, 24)]

        def bcast(src, d):
            return lax.concatenate([lax.broadcast_in_dim(src[d:d + 1, t:t + LANES], (8, LANES), (0, 1))
                                    for t in range(0, BQ, LANES)], 1)

        def row_groups(*xs):
            return [(x, r) for x in xs for r in range(0, x.shape[0], 8)]

        def key_products(bwd, slab, c, st, w):
            mxu = _dot(vk[tile(c, CK, CK - 8 * VG[bwd][c % 2], w.shape[0])], w)
            tokens = st.get("prev", [None] * PACE[bwd][1]) + row_groups(mxu)
            ops = [(p, g, d) for p in range(2) for d in range(DH) for g in range(VG[bwd][p])]
            if c == 0:
                st["rows"] = [bcast(slab, d) for d in list(range(DH)) + [23] * bwd]
            for n, (p, g, d) in enumerate(ops):
                step, phase = divmod(2 * n, len(ops))
                if step != c % 2:
                    continue
                blk_i, cc = divmod(c - c % 2 + p, BQ // CK)
                k = vkb[tile(blk_i * _table_tiles() + _vpu_groups().index((bwd, cc, g)) * DH + d, 8)]
                token = tokens[min(PACE[bwd][0] + phase * PACE[bwd][1] // len(ops), len(tokens) - 1)]
                if token and (d + bwd) % st.get("every", 2) == 0:
                    x, r = token
                    k = lax.select(st["never"], lax.slice(x, (r, 0), (r + 8, LANES)), k)
                t = _wide(k) * st["rows"][d]
                st[p, g] = st[p, g] + t if d else (st["rows"][DH] + t if bwd else t)
            return jnp.concatenate([mxu] + [st[c % 2, g] for g in range(VG[bwd][c % 2])], axis=0), mxu

        def q_weights(q):
            return jnp.concatenate([jnp.zeros((24, BQ), F32), q[...]], axis=0).astype(BF)

        def scores(h, par, c, st):
            if "never" in st:
                if c == 0:
                    st["w"] = q_weights(head(ql, h))
                s, mxu = key_products(0, head(ql, h), c, st, st["w"])
            else:
                s = mxu = _dot(vk[tile(c, CK, CK, 48)], st["w"])
            s_s[par][c * CK:(c + 1) * CK] = s
            m = jnp.max(s.reshape(CK // 8, 8, BQ), axis=0)
            st["m"] = jnp.maximum(st["m"], m) if c else m
            return mxu

        def weigh(h, par, c, mrow, acc):
            e = jnp.exp2(s_s[par][c * CK:(c + 1) * CK] - jnp.concatenate([mrow] * (CK // 8), axis=0)).astype(BF)
            e_s.at[_ds(h * (S // 2), S // 2)][c * CK // 2:(c + 1) * CK // 2] = pltpu.bitcast(e, U32)
            o = _dot(vt[tile(c, 24)], e)
            return (o if acc is None else acc + o), o

        def fwd_head(h, par, carry, st, first=False):
            m, mrow, acc = carry
            for c in range(NC):
                done = [scores(h + 1, 1 - par, c, st)]
                if c:
                    acc, o = weigh(h, par, c - 1, mrow, acc if c > 1 else None)
                    done.append(o)
                else:
                    if not first:
                        ol[_ds((h - 1) * 24, 24)], o = weigh(h - 1, 1 - par, NC - 1, mrow, acc)
                        done.append(o)
                    mrow = jnp.broadcast_to(jnp.max(m, axis=0, keepdims=True), (8, BQ))
                st["prev"] = row_groups(*done)
            return st["m"], mrow, acc

        def fwd_group(i, j, carry):
            @pl.when(jnp.logical_and(i == 0, j == 1))
            def _():
                for cp in mod_in[2:5]:
                    cp.start()

            @pl.when(jnp.logical_and(i == 0, j == 2))
            def _():
                for n in range(2, 5):
                    mod_in[n].wait()
                for n in range(2, 5):
                    set_mod(n, wbuf[n * D:(n + 1) * D])
                for cp in late_in:
                    cp.start()

            st = {"never": j < 0}
            for u in range(1, UF + 1):
                carry = fwd_head(j * UF + u, u % 2, carry, st)
            return carry

        def bwd_tail(h, c, ds, acc):
            gk = _dot(head(ql, h)[...], ds, NT)
            dkt[tile(c, 24)] += gk
            o = _dot(kt[tile(c, 24)], ds)
            acc = acc + o if c else o
            if c == NC - 1:
                dql[_ds(h * 24, 24)] = pltpu.bitcast(acc, U32)
            return acc, gk, o

        def store_dq(i, j):
            slabs = dql.at[_ds(j * UB * 24, UB * 24)]
            heads = [pltpu.bitcast(slabs[u * 24:(u + 1) * 24], F32) for u in range(UB)]
            dqt[_ds(i * (D // 2) + j * (UB * DH // 2), UB * DH // 2)] = _pack(_join_heads(heads) * DH ** -0.5)

        def bwd_group(i, j, acc):
            @pl.when(j == 1)
            def _():
                o_copy(i).start()

                @pl.when(i == NB - 1)
                def _():
                    for cp in early_out:
                        cp.start()

            @pl.when(j == H // UB // 2)
            def _():
                o_copy(i).wait()

                @pl.when(i < NB - 1)
                def _():
                    g_copy(i + 1).start()

                @pl.when(i == NB - 1)
                def _():
                    for cp in early_out:
                        cp.wait()
                    for cp in mod_in:
                        cp.start()

            st = {"never": j < 0}
            ds = pltpu.bitcast(s_b[0:CK // 2], BF)
            for u in range(UB):
                h = j * UB + u
                do = head(ol, h)
                w = jnp.concatenate([do[...], jnp.zeros((8, BQ), F32)], axis=0).astype(BF)
                for c in range(NC):
                    dp, mxu = key_products(1, do, c, st, w)
                    e = _unpack(e_s.at[_ds(h * (S // 2), S // 2)][c * CK // 2:(c + 1) * CK // 2])
                    gv = _dot(do[...], e, NT)
                    dvt[tile(c, 24)] += gv
                    if c:
                        acc, gk, gq = bwd_tail(h, c - 1, ds, acc)
                    else:
                        acc, gk, gq = bwd_tail(jnp.maximum(h - 1, 0), NC - 1, ds, acc)
                    st["prev"] = row_groups(mxu, gv, gk, gq)
                    if (u, c) == (0, 1):
                        store_dq(i, jnp.maximum(j - 1, 0))
                    ds = (e.astype(F32) * dp).astype(BF)
            s_b[0:CK // 2] = pltpu.bitcast(ds, F32)
            return acc

        def mid(i, carry, df_split):
            attn_s, x1_s = (s_b.at[pl.ds(n * D, D)] for n in range(2))
            tmp_s, dat = s_a, dqt.at[blk(i)]
            st = {"acc": None}
            m, mrow, acc = carry
            ol[(H - 2) * 24:(H - 1) * 24] = weigh(H - 2, 0, NC - 1, mrow, acc)[0]
            mrow = jnp.broadcast_to(jnp.max(m, axis=0, keepdims=True), (8, BQ))

            def paced(x, step=2):
                token = st["tokens"][0]
                st["tokens"] = st["tokens"][step:] or st["tokens"][-1:]
                token = token[0:8, :LANES]
                if jnp.result_type(x) == U32:
                    token = pltpu.bitcast(token, U32)
                return jnp.where(i < 0, _wide(token[0:1]), x)

            def prepare(split):
                return (lambda r: split.prepare(r, lambda words: paced(words, 1))), split.steps

            def fence():
                @pl.loop(0, i // NB)
                def _(_):
                    s_b[S - 8:S] = jnp.zeros((8, BQ), F32)

            def last_head(c):
                st["acc"] = weigh(H - 1, 1, c, mrow, st["acc"])[0]

            def o_norm(n):
                heads = [ol[h * 24:(h + 1) * 24] for h in range(4 * n, 4 * n + 4)]
                obt[n * 2 * DH:(n + 1) * 2 * DH] = _pack(_join_heads([a * (1.0 / a[DH:DH + 1]) for a in heads]))

            def o_proj(r):
                attn = _dot(wo[:, r], _unpack(obt[...]), TN)
                attn_s[r] = attn
                x1 = _unpack(xt[blk(i, r)]).astype(F32) + _wide(modc[2, r]) * attn
                x1_s[r] = x1
                accumulate(st, "sum", x1)

            def ln2_var(r):
                xc = x1_s[r] - paced(st["mu"])
                accumulate(st, "var", xc * xc)

            def ln2_out(r):
                xh2 = (x1_s[r] - paced(st["mu"])) * st["rstd"]
                h2t[half(r)] = _pack(xh2 * _wide(modc[4, r]) + _wide(modc[3, r]))

            def d_act(rs):
                for r, da in zip(rs, df_split(w2[rs[0]], w2[rs[1]])):
                    tmp_s[r] = da
                st["tokens"] = df_split.products

            def act(rs):
                todo = st.pop("act", [])
                if rs:
                    st["act"] = list(zip(rs, st["h2"](w1t[rs[0]], w1t[rs[1]])))
                    st["tokens"] = st["h2"].products
                for r, pre in todo:
                    for k in range(0, MA, 16):
                        u, rows = pre[k:k + 16], slice(r.start + k, r.start + k + 16)
                        sg = 0.5 * jnp.tanh(paced(0.5, 1) * u) + 0.5
                        a = u * sg
                        at[half(rows)] = _pack(a)
                        dut[half(rows)] = _pack(tmp_s[rows] * (sg + a * (1.0 - sg)))

            def over_hidden(w, x, r):
                st["tokens"] = [_dot(w[k, r], _unpack(x[half(k)]), TN) for k in _chunks(F, KC)]
                return sum(st["tokens"][1:], st["tokens"][0])

            def d_h2(r):
                dh2 = over_hidden(w1t, dut, r)
                t = dh2 * ((x1_s[r] - st["mu"]) * st["rstd"])
                dmodc[3, r] += _fold(dh2)
                dmodc[4, r] += _fold(t)
                cb = _wide(modc[4, r])
                dy = dh2 * cb
                tmp_s[r] = dy
                accumulate(st, "m1", dy)
                accumulate(st, "m2", t * cb)

            def ffn_out(r):
                f = over_hidden(w2, at, r)
                dmodc[5, r] += _fold(_unpack(gt[half(r)]).astype(F32) * f)
                o_out[:, r] = (x1_s[r] + _wide(modc[5, r]) * f).astype(BF).T

            def ln2_bwd(r):
                dx1 = _unpack(gt[half(r)]).astype(F32) + st["rstd"] * (
                    tmp_s[r] - paced(st["m1"], 0) - (x1_s[r] - st["mu"]) * paced(st["m2"], 1))
                dx1t[blk(i, r)] = _pack(dx1)
                dmodc[2, r] += _fold(dx1 * attn_s[r])
                dat[half(r)] = _pack(dx1 * _wide(modc[2, r]))

            def d_o(rs):
                for r, do in zip(rs, st["da"](wo[rs[0]], wo[rs[1]])):
                    tmp_s[r] = do

            def do_prep(h):
                r24 = _rows(24, BQ)
                o = ol[h * 24:(h + 1) * 24]
                inv = 1.0 / paced(o[DH:DH + 1])
                d = (_head_rows(tmp_s, h) * inv).astype(BF).astype(F32)
                delta = _colsum(jnp.where(r24 < DH, d * o, 0.0)) * inv
                d0 = delta.astype(BF).astype(F32)
                d1 = (delta - d0).astype(BF).astype(F32)
                r8 = _rows(8, BQ)
                tail = jnp.where(r8 < 4, d[16:24], jnp.where(r8 == 4, d0, jnp.where(
                    r8 == 5, d1, jnp.where(r8 == 6, delta - d0 - d1, -delta))))
                ol[h * 24:(h + 1) * 24] = jnp.concatenate([d[0:16], tail], axis=0)

            def w_grad(acc, out, lhs, rhs):
                def step(rs):
                    for r, g in zip(rs, rhs(*(_unpack(lhs[half(r)]) for r in rs))):
                        g = acc[r] + g
                        acc[r] = g
                        out[r] = jnp.where(i == NB - 1, g.astype(BF), out[r])
                    st["tokens"] = rhs.products
                return step

            fine, fch = _pairs(F, MA), _pairs(F, FC)
            _mix((d_act, fine[:7]), (last_head, range(NC)), (o_norm, range(H // 4 - 1)))
            ol[(H - 1) * 24:H * 24] = st["acc"]
            _mix((d_act, fine[7:8]), (o_norm, [H // 4 - 1]))
            _mix((o_proj, dch))
            st["mu"] = _colsum(st["sum"]) * inv_d
            _mix((d_act, fine[8:10]), (ln2_var, dch))
            st["rstd"] = lax.rsqrt(_colsum(st["var"]) * inv_d + EPS)
            _mix((d_act, fine[10:16]), (ln2_out, _chunks(D, 32)))
            st["h2"] = _Split(h2t, sum_b, NN)
            _mix((d_act, fine[16:]), (st["h2"].prepare, _Split.steps))
            _mix((act, fine))

            fence()
            act(None)
            for_w2, for_w1, for_wo = _Split(dft, sum_c, NT), _Split(h2t, sum_b, NT), _Split(dat, sum_a, NT)
            _mix((d_h2, dch[:-1]), prepare(for_w2), prepare(for_w1))
            d_h2(dch[-1])
            st["m1"] = _colsum(st["m1"]) * inv_d
            st["m2"] = _colsum(st["m2"]) * inv_d * st["rstd"]
            st["tokens"] = [st["m1"]]
            _mix((ln2_bwd, _chunks(D, 16)), (ffn_out, lch[:-1]))
            st["da"] = _Split(dat, sum_a, NN)
            _mix((st["da"].prepare, _Split.steps))
            ffn_out(lch[-1])
            _mix((d_o, _pairs(D, MO)))

            fence()
            _mix((w_grad(dw1_acc, w1t, dut, for_w1), fch), (do_prep, range(H // 2)), prepare(for_wo))
            _mix((w_grad(dw2_acc, w2, at, for_w2), fch), (do_prep, range(H // 2, H)))
            s_b[0:CK // 2] = jnp.zeros((CK // 2, BQ), F32)
            _mix((w_grad(dwo_acc, wo, obt, for_wo), _pairs(D, D // 4)))

        finish, in_flight = epilogue(dwq, dx_out, obt)

        def block(i, carry):
            g_copy(i).wait()
            for r in dch:
                gb = g_in[:, r].T
                gt[half(r)] = pltpu.bitcast(gb, U32)
                df = gb.astype(F32) * _wide(modc[5, r])
                dft[half(r)] = _pack(df)
                q = _dot(wq[:, r], _unpack(h1t[blk(i)]), TN)
                s_b[r] = jnp.where(i < 0, df, q * qscale).astype(BF).astype(F32)
            df_split = _Split(dft, sum_a, NN)
            _mix((df_split.prepare, _Split.steps))
            st = {}
            for c in range(NC):
                for h in range(c * H // NC, (c + 1) * H // NC):
                    ql[h * 24:(h + 1) * 24] = _head_rows(s_b, h)
                st["w"] = q_weights(head(ql, i // NB))
                st["prev"] = row_groups(scores(0, 0, c, st))
            st.update(never=i < 0, every=1)
            m = fwd_head(0, 0, (st["m"], None, None), st, first=True)
            m = lax.fori_loop(0, (H - 2) // UF, lambda j, m: fwd_group(i, j, m), m)

            @pl.when(i == 0)
            def _():
                for cp in late_in:
                    cp.wait()

            mid(i, m, df_split)

            acc = lax.fori_loop(0, H // UB, lambda j, a: bwd_group(i, j, a), jnp.zeros((24, BQ), F32))
            bwd_tail(H - 1, NC - 1, pltpu.bitcast(s_b[0:CK // 2], BF), acc)
            store_dq(i, H // UB - 1)

            @pl.when(i == NB - 1)
            def _():
                for cp in mod_in:
                    cp.wait()
                finish()

            return carry

        lax.fori_loop(0, NB, block, 0)
        for cp in in_flight:
            cp.wait()

    packed = lambda rows: pltpu.VMEM((rows // 2, BQ), U32)
    pl.run_scoped(
        main,
        packed(F), packed(F),
        *[packed(D)] * 4,
        *[pltpu.VMEM((HB // 2, 5 * HB), U32)] * 3,
        pltpu.VMEM((D, D), BF), pltpu.VMEM((2, BQ, D), BF),
    )


def _scratch_shapes(S, D, F):
    NB = S // BQ
    return [
        pltpu.VMEM((NB * D // 2, BQ), U32),
        pltpu.VMEM((NB * D // 2, BQ), U32),
        pltpu.VMEM((NB, 2, 8, BQ), F32),
        pltpu.VMEM((NB * D // 2, BQ), U32),
        pltpu.VMEM((NB * D // 2, BQ), U32),
        pltpu.VMEM((sum(_arena_rows(S)), BQ), F32),
        pltpu.VMEM((H * S // 2, BQ), U32),
        pltpu.VMEM((H * 24, BQ), F32),
        pltpu.VMEM((H * 24, BQ), F32),
        pltpu.VMEM((6, D, LANES), F32),
        pltpu.VMEM((6, D, LANES), F32),
        pltpu.VMEM((D, D), BF),
        pltpu.VMEM((max(D + 2 * F, 6 * D), D), BF),
        pltpu.VMEM((D, D), F32), pltpu.VMEM((F, D), F32), pltpu.VMEM((F, D), F32),
        pltpu.VMEM((BQ, D), BF),
        pltpu.VMEM((16, D), F32),
        pltpu.VMEM((DH, D), BF), pltpu.VMEM((DH, D), BF), pltpu.VMEM((1, D), BF),
        pltpu.SemaphoreType.DMA((16,)),
    ]


@jax.jit
def pallas_adaLN_cond__grouped_kv_mqa__dense_activation_silu__prompt_kernel(
    A_x: jax.Array,
    A_wq: jax.Array,
    A_wk: jax.Array,
    A_wv: jax.Array,
    A_wo: jax.Array,
    B_x: jax.Array,
    B_w1: jax.Array,
    B_w2: jax.Array,
    c: jax.Array,
    w_mod: jax.Array,
    grad_out: jax.Array,
):
    del B_x
    _, S, D = A_x.shape
    F = B_w2.shape[0]
    hbm = pl.BlockSpec(memory_space=pl.ANY)
    sds = lambda *shape: jax.ShapeDtypeStruct(shape, BF)

    out, dx, dwq, dwo, dw1t, dw2, dwmod, dwkt, dwvt, dc = pl.pallas_call(
        _kernel,
        in_specs=[hbm] * 10,
        out_specs=[hbm] * 10,
        out_shape=[sds(S, D), sds(S, D), sds(D, D), sds(D, D), sds(F, D), sds(F, D), sds(D, 6 * D),
                   sds(DH, D), sds(DH, D), sds(1, D)],
        scratch_shapes=_scratch_shapes(S, D, F),
        compiler_params=pltpu.CompilerParams(vmem_limit_bytes=128 * 1024 * 1024),
        name="adaln_mqa_silu_fwd_bwd",
    )(A_x.reshape(S, D), grad_out.reshape(S, D), A_wq, A_wo, B_w1.T, B_w2, w_mod, A_wk.T, A_wv.T, c)
    return (out.reshape(A_x.shape), dx.reshape(A_x.shape), dwq, dwkt.T, dwvt.T, dwo, dw1t.T, dw2, dc, dwmod)
```
